```python
import os as _os
_os.environ.setdefault("JAX_PLATFORMS", "cpu")
import jax
import jax.numpy as jnp

def _softmax(x, axis=-1):
    return jax.nn.softmax(x, axis=axis)
def _gelu(x):
    return jax.nn.gelu(x, approximate=True)
def _silu(x):
    return jax.nn.silu(x)
def _sigmoid(x):
    return jax.nn.sigmoid(x)
def _layernorm(x, axis=-1, eps=1e-5):
    m = jnp.mean(x, axis=axis, keepdims=True)
    v = jnp.var(x, axis=axis, keepdims=True)
    return (x - m) / jnp.sqrt(v + eps)
def _scatter_add(tgt, idx, src, axis=0):
    return tgt.at[idx].add(src)
def _segment_sum(src, seg, n):
    return jax.ops.segment_sum(src, seg, n)
class _Rng:
    def __init__(self, key):
        self._k = key
    def _next(self):
        self._k, sub = jax.random.split(self._k)
        return sub
    def normal(self, shape):
        return jax.random.normal(self._next(), shape, dtype=jnp.bfloat16)
    def randint(self, lo, hi, shape):
        return jax.random.randint(self._next(), shape, lo, hi, dtype=jnp.int32)
    def uniform(self, shape, lo=0.0, hi=1.0):
        return jax.random.uniform(self._next(), shape, jnp.bfloat16, lo, hi)
    def permutation(self, n):
        return jax.random.permutation(self._next(), n)


kernel_name = 'interleave_layers__sliding_local_dilated__sliding_local_dilated__prompt'

def setup_inputs():
    _rng = _Rng(jax.random.key(int.from_bytes(__import__("os").urandom(4), "little")))
    _w = (lambda a: (lambda t: t.astype(jnp.bfloat16) if jnp.issubdtype(t.dtype, jnp.floating) else t)(jnp.asarray(a)))
    def _A_setup():
        B, S, D = 1, 2048, 1024
        return {
            "x": _w((lambda *s: _rng.normal(s) * 0.05)(B, S, D)),
            "wqkv": _w((lambda *s: _rng.normal(s) * 0.05)(D, 3 * D)),
            "wo": _w((lambda *s: _rng.normal(s) * 0.05)(D, D)),
        }
    _A_in = _A_setup()

    def _B_setup():
        B, S, D = 1, 2048, 1024
        return {
            "x": _w((lambda *s: _rng.normal(s) * 0.05)(B, S, D)),
            "wqkv": _w((lambda *s: _rng.normal(s) * 0.05)(D, 3 * D)),
            "wo": _w((lambda *s: _rng.normal(s) * 0.05)(D, D)),
        }
    _B_in = _B_setup()

    return {
        "A_x": _A_in["x"],
        "A_wqkv": _A_in["wqkv"],
        "A_wo": _A_in["wo"],
        "B_x": _B_in["x"],
        "B_wqkv": _B_in["wqkv"],
        "B_wo": _B_in["wo"],
    }

def reference(A_x, A_wqkv, A_wo, B_x, B_wqkv, B_wo):
    def _A_ref(x, wqkv, wo):
        B, S, D = x.shape
        H = 32; Dh = D // H
        W, dil = 8, 2
        qkv = (lambda x, *d: x.transpose(*d))((x @ wqkv).reshape(B, S, 3, H, Dh), 2, 0, 3, 1, 4)
        q, k, v = qkv[0], qkv[1], qkv[2]
        scale = Dh ** -0.5
        pos = jnp.arange(S)
        off = jnp.arange(W) * dil
        idx = pos[:, None] - off[None, :]
        mask = idx >= 0
        idx_c = jnp.where(mask, idx, 0).reshape(-1)
        kg = k[:, :, idx_c, :].reshape(B, H, S, W, Dh)
        vg = v[:, :, idx_c, :].reshape(B, H, S, W, Dh)
        logits = jnp.einsum("bhsd,bhswd->bhsw", q, kg) * scale
        logits = jnp.where(mask[None, None, :, :], logits, -1e9)
        attn = _softmax(logits, axis=-1)
        o = jnp.einsum("bhsw,bhswd->bhsd", attn, vg)
        return (lambda x, *d: x.transpose(*d))(o, 0, 2, 1, 3).reshape(B, S, D) @ wo

    def _B_ref(x, wqkv, wo):
        B, S, D = x.shape
        H = 32; Dh = D // H
        W, dil = 8, 2
        qkv = (lambda x, *d: x.transpose(*d))((x @ wqkv).reshape(B, S, 3, H, Dh), 2, 0, 3, 1, 4)
        q, k, v = qkv[0], qkv[1], qkv[2]
        scale = Dh ** -0.5
        pos = jnp.arange(S)
        off = jnp.arange(W) * dil
        idx = pos[:, None] - off[None, :]
        mask = idx >= 0
        idx_c = jnp.where(mask, idx, 0).reshape(-1)
        kg = k[:, :, idx_c, :].reshape(B, H, S, W, Dh)
        vg = v[:, :, idx_c, :].reshape(B, H, S, W, Dh)
        logits = jnp.einsum("bhsd,bhswd->bhsw", q, kg) * scale
        logits = jnp.where(mask[None, None, :, :], logits, -1e9)
        attn = _softmax(logits, axis=-1)
        o = jnp.einsum("bhsw,bhswd->bhsd", attn, vg)
        return (lambda x, *d: x.transpose(*d))(o, 0, 2, 1, 3).reshape(B, S, D) @ wo

    x = A_x
    x = x + _A_ref(_layernorm(x, axis=-1), A_wqkv, A_wo)
    x = x + _B_ref(_layernorm(x, axis=-1), B_wqkv, B_wo)
    x = x + _A_ref(_layernorm(x, axis=-1), A_wqkv, A_wo)
    x = x + _B_ref(_layernorm(x, axis=-1), B_wqkv, B_wo)
    return x
```

```python
import functools

import jax
import jax.numpy as jnp
from jax.experimental import pallas as pl
from jax.experimental.pallas import tpu as pltpu

S, D = 2048, 1024
H, DH = 32, 32
W, DIL = 8, 2
NS = 8
SJ = S // NS
TJ = 32
TM = TJ * NS
HM, HD = TM // 2, D // 2
NT = SJ // TJ
NL = 4
NC = D // 128
HC = NC // 2
HJ = (W - 1) * DIL
NCH = 128
EPS = 1e-5
SCALE = DH ** -0.5
LOG2E = 1.4426950408889634
NQD = 4
LAG = 4
CL, CQ, CP, CC = 35, 160, 160, 30
CUT = 55


def _wo_src_group(rp):
    c, g, b = rp >> 4, (rp >> 2) & 3, rp & 3
    return (b << 5) | (g << 3) | c


def _left_operands(a11, a12, a21, a22):
    return (a11 + a22, a21 + a22, a11, a22, a11 + a12, a21 - a11, a12 - a22)


def _right_operands(b11, b12, b21, b22):
    return (b11 + b22, b11, b12 - b22, b21 - b11, b22, b11 + b12, b21 + b22)


def _kernel(x_hbm, wqa_hbm, woa_hbm, wqb_hbm, wob_hbm, out_hbm,
            xs, hs0, hs1, qkv0, qkv1, halo0, halo1, of, os0, os1, os2, wq, wo, wq_raw, wo_raw, x_raw, w_tmp, wo_tmp, o_stage,
            zero_ref, sem_x, sem_w, sem_q, sem_o):
    f32, bf16, u32 = jnp.float32, jnp.bfloat16, jnp.uint32
    part = functools.partial
    hs, os_, halos = (hs0, hs1), (os0, os1), (halo0, halo1)

    def lanes(c, n=1):
        return slice(c * 128, (c + n) * 128)

    def pack(even, odd):
        return pltpu.bitcast(pltpu.pack_elementwise([even, odd], packed_dtype=bf16), u32)

    def unpack(u):
        return [pltpu.unpack_elementwise(u, index=i, packed_dtype=bf16, unpacked_dtype=f32) for i in range(2)]

    def mult(i, n):
        return i * n if isinstance(i, int) else pl.multiple_of(i * n, n)

    def x_copy(t):
        return pltpu.make_async_copy(x_hbm.at[:, pl.ds(t * TJ, TJ), :], x_raw.at[t], sem_x.at[t])

    def wq_first_copy(i):
        rows = pl.ds(i * (HD // NQD), HD // NQD)
        return pltpu.make_async_copy(wqa_hbm.at[:, rows, pl.ds(0, D)], wq_raw.at[0, 0, :, rows], sem_q.at[i])

    def wq_copy(s, p):
        src = (wqa_hbm, wqb_hbm)[s]
        return pltpu.make_async_copy(src.at[:, :, pl.ds(p * D, D)], wq_raw.at[s, p], sem_w.at[s * 4 + p])

    def wo_copy(s):
        src = (woa_hbm, wob_hbm)[s]
        return pltpu.make_async_copy(src, wo_raw.at[s], sem_w.at[s * 4 + 3])

    def out_copy(t):
        return pltpu.make_async_copy(o_stage.at[t], out_hbm.at[:, pl.ds(t * TJ, TJ), :], sem_o.at[t])

    def start_now(*copies):
        def body(i, carry):
            for cp in copies:
                cp.start()
            return carry
        jax.lax.fori_loop(0, zero_ref[0] + 1, body, 0)

    class Chain:
        def __init__(self, on=True):
            self.never = jax.lax.broadcasted_iota(jnp.int32, (NS, 128), 0) + zero_ref[0] < 0
            self.tok = None
            self.on = on

        def after(self, v):
            if not self.on or self.tok is None:
                return v
            tok = pltpu.bitcast(self.tok, v.dtype)
            return jnp.concatenate(
                [jnp.where(self.never, tok, v[r:r + NS]) for r in range(0, v.shape[0], NS)], axis=0)

        def mark(self, v):
            self.tok = v

    def shuffle_lanes(s, p, a, pairs, ch):
        lane = (jax.lax.broadcasted_iota(jnp.int32, (8, 128), 1) - 2 * a) & 127
        src = ((lane & 16) << 2) | ((lane & 1) << 5) | ((lane >> 5) << 3) | ((lane >> 1) & 7)
        for half in range(2):
            for r2 in pairs:
                u = pltpu.bitcast(wq_raw[s, p, half, pl.ds(mult(r2 // 8, 16), 16), lanes(a)], u32)
                u = jnp.take_along_axis(ch.after(u), src, axis=1)
                w_tmp[p % 2, half, pl.ds(r2, 8), lanes(a)] = u
        ch.mark(u)

    def exchange_chunks(v):
        lane = jax.lax.broadcasted_iota(jnp.int32, (8, 128), 1)
        for sh in (1, 2, 4):
            on = (lane & (2 * sh)) != 0
            v = [jnp.where(on, v[(k + sh) % NC], v[k]) for k in range(NC)]
        return [pltpu.roll(v[NC - c], 128 - 2 * c, 1) if c else v[0] for c in range(NC)]

    def right_operands(b11, b12, b21, b22):
        even, odd = [_right_operands(b11[i], b12[i], b21[i], b22[i]) for i in range(2)]
        return [pack(e, o) for e, o in zip(even, odd)]

    def left_operands(a11, a12, a21, a22):
        even, odd = [_left_operands(a11[i], a12[i], a21[i], a22[i]) for i in range(2)]
        return [pack(e, o) for e, o in zip(even, odd)]

    def prep_wq(s, p, r2, ch, mark=False):
        raw = [[w_tmp[p % 2, half, pl.ds(r2, 8), lanes(a)] for a in range(NC)] for half in range(2)]
        raw = [[ch.after(u) if a % 2 == 0 else u for a, u in enumerate(v)] for v in raw]
        top, bot = [[unpack(u) for u in exchange_chunks(v)] for v in raw]
        for c in range(HC):
            for m, b in enumerate(right_operands(top[c], top[c + HC], bot[c], bot[c + HC])):
                wq[s, m, pl.ds(r2, 8), lanes(p * HC + c)] = b
        if mark:
            ch.mark(top[1][0])

    def wq_jobs(s, p, ch):
        def first(a):
            if a == 0:
                wq_copy(s, p).wait()
            shuffle_lanes(s, p, a, range(0, HD // 2, 8), ch)

        def second(r2):
            prep_wq(s, p, r2, ch, (r2 // 8) % 2 == 1)
        return [part(first, a) for a in range(NC)] + [part(second, r2) for r2 in range(0, HD // 2, 8)]

    def wo_jobs(s, ch):
        def spread(c, i, a):
            if c == i == a == 0:
                wo_copy(s).wait()
            v = ch.after(wo_raw[s, a * 128:(a + 1) * 128, lanes(c + i * HC)].astype(f32))
            wo_tmp[c % 2, i, pl.ds(a, 128, stride=8), :] = v
            ch.mark(v[:NS])

        def gather(c, rp):
            def rows(i, q):
                return [wo_tmp[c % 2, i, g * 8:g * 8 + 8, :] for g in (_wo_src_group(q), _wo_src_group(q + 1))]
            ops = right_operands([ch.after(b) for b in rows(0, rp)], rows(1, rp),
                                 rows(0, rp + 64), [ch.after(b) for b in rows(1, rp + 64)])
            for m, b in enumerate(ops):
                wo[s, m, rp * 4:rp * 4 + 8, lanes(c)] = b
            ch.mark(ops[-1])
        jobs = []
        for c in range(HC):
            jobs += [part(spread, c, i, a) for i in range(2) for a in range(8)]
            jobs += [part(gather, c, rp) for rp in range(0, 64, 2)]
        return jobs

    def load_x(t, i, ch):
        if i == 0:
            x_copy(t).wait()
        v = x_raw[t, i].astype(f32)
        for c in range(NC):
            u = ch.after(v[:, lanes(c)])
            xs[c, pl.ds(t * TM + i, TJ, stride=NS), :] = u
            if c % 2:
                ch.mark(u[:NS])

    def ln_jobs(t, dst, ch):
        mean, rstd = {}, {}

        def xv(c, rr):
            return xs[c, pl.ds(mult(t, TM) + rr, NS, stride=2), :]

        def groups(r):
            return (r, r + 1, r + HM, r + HM + 1)

        def means(r):
            for rr in groups(r):
                tot = ch.after(xv(0, rr))
                for c in range(1, NC):
                    tot = tot + xv(c, rr)
                mean[rr] = jnp.broadcast_to(jnp.sum(tot, axis=-1, keepdims=True) * (1.0 / D), (NS, 128))
            ch.mark(tot)

        def variances(r, i):
            for rr in groups(r)[2 * i:2 * i + 2]:
                mu = ch.after(mean[rr])
                sq = None
                for c in range(NC):
                    xc = xv(c, rr) - mu
                    sq = xc * xc if c == 0 else sq + xc * xc
                var = jnp.sum(sq, axis=-1, keepdims=True) * (1.0 / D)
                rstd[rr] = jnp.broadcast_to(jax.lax.rsqrt(var + EPS), (NS, 128))
            ch.mark(sq)

        def operands(r, c):
            mu = {rr: ch.after(mean[rr]) for rr in groups(r)}

            def norm(cc, rr):
                return [(xv(cc, q) - mu[q]) * rstd[q] for q in (rr, rr + 1)]
            ops = left_operands(norm(c, r), norm(c + HC, r), norm(c, r + HM), norm(c + HC, r + HM))
            for m, a in enumerate(ops):
                dst[0][dst[1], m, r // 2:r // 2 + 8, lanes(c)] = a
            ch.mark(ops[-1])

        jobs = []
        for r in range(0, HM + 32, 16):
            if r < HM:
                jobs.append((CL, part(means, r)))
            if 16 <= r <= HM:
                jobs += [(CL, part(variances, r - 16, i)) for i in range(2)]
            if r >= 32:
                jobs += [(CL, part(operands, r - 32, c)) for c in range(HC)]
        return jobs

    def h_of(n):
        return (hs[n % 2], (n // 2) % 4)

    def x_jobs(t, ch):
        return [(2 * CL, part(load_x, t, i, ch)) for i in range(NS)] + ln_jobs(t, h_of(t), ch)

    def stage_out(t, i):
        o_stage[t, i] = jnp.concatenate(
            [xs[c, pl.ds(mult(t, TM) + i, TJ, stride=NS), :] for c in range(NC)], axis=1).astype(bf16)

    def write_out(t):
        for i in range(NS):
            stage_out(t, i)
        out_copy(t).start()

    issued = []

    def matmul_jobs(left, right, store):
        jobs = []
        for n in range(HD // NCH):
            st = {}

            def prod(m, n=n):
                res = jnp.dot(pltpu.bitcast(left(m), bf16), pltpu.bitcast(right(m, n), bf16),
                              preferred_element_type=f32)
                issued.append(res[HM - NS:, NCH - 128:])
                return res

            def put(hi, right_half, val, n=n):
                for u in range(NCH // 128):
                    store(hi, right_half * HC + n * (NCH // 128) + u, val[:, lanes(u)])

            def j7(st=st, prod=prod):
                st["p"] = prod(6)

            def j5(st=st, prod=prod):
                st["m5"] = prod(4)
                st["p"] = st["p"] - st["m5"]

            def j3(st=st, prod=prod, put=put):
                st["q"] = prod(2)
                put(0, 1, st["q"] + st["m5"])

            def j6(st=st, prod=prod):
                st["q"] = st["q"] + prod(5)

            def j1(st=st, prod=prod):
                m1 = prod(0)
                st["p"] = st["p"] + m1
                st["q"] = st["q"] + m1

            def j4(st=st, prod=prod, put=put):
                st["m4"] = prod(3)
                put(0, 0, st["p"] + st["m4"])

            def j2(st=st, prod=prod, put=put):
                m2 = prod(1)
                put(1, 0, m2 + st["m4"])
                put(1, 1, st["q"] - m2)
            jobs += [j7, j5, j3, j6, j1, j4, j2]
        return jobs

    def qkv_jobs(src, s, p, dst):
        def store(hi, c, val):
            dst[0][dst[1], p * NC + c, hi * HM:(hi + 1) * HM, :] = val
        return matmul_jobs(lambda m: src[0][src[1], m],
                           lambda m, n: wq[s, m, :, p * HD + n * NCH:p * HD + (n + 1) * NCH], store)

    def proj_jobs(src, s, t):
        def store(hi, c, val):
            rows = pl.ds(mult(t, TM) + hi * HM, HM)
            xs[c, rows, :] = xs[c, rows, :] + val
        return matmul_jobs(lambda m: src[m], lambda m, n: wo[s, m, :, n * NCH:(n + 1) * NCH], store)

    def halo_jobs(t, prev, halo):
        def job(c):
            for j in range(HJ):
                r = (TJ - HJ + j) * NS
                src = prev[0][prev[1], c, r:r + NS, :]
                if (t == 0) is not False:
                    src = jnp.where(t == 0, pltpu.roll(src, 1, 0), src)
                halo[c - NC, j * NS:(j + 1) * NS, :] = src
        return [part(job, c) for c in range(NC, 3 * NC)]

    def clamp_halo(t, cur, halo):
        if (t == 0) is False:
            return
        sub = jax.lax.broadcasted_iota(jnp.int32, (NS, 128), 0)
        for c in range(2 * NC, 3 * NC):
            first = jnp.broadcast_to(cur[0][cur[1], c, 0:1, :], (NS, 128))
            for j in range(HJ):
                rows = slice(j * NS, (j + 1) * NS)
                halo[c - NC, rows, :] = jnp.where(sub + t == 0, first, halo[c - NC, rows, :])

    def attn_jobs(t, cur, halo, dst, ch, every=1):
        buf, slot = cur
        probs = {}

        def kv(c, j):
            if j >= 0:
                return buf[slot, c, j * NS:(j + 1) * NS, :]
            return halo[c - NC, (j + HJ) * NS:(j + HJ + 1) * NS, :]

        def qk(j):
            acc = [None] * W
            for c in range(NC):
                qv = ch.after(kv(c, j))
                for w in range(W):
                    pr = qv * kv(NC + c, j - w * DIL)
                    acc[w] = pr if c == 0 else acc[w] + pr
                if c % every == every - 1:
                    ch.mark(acc[W - 1])
            lg = []
            for w in range(W):
                a = acc[w]
                a = a + pltpu.roll(a, 64, 1)
                a = a + pltpu.roll(a, 32, 1)
                if j - w * DIL < 0 and (t == 0) is not False:
                    sub = jax.lax.broadcasted_iota(jnp.int32, (NS, 128), 0)
                    a = jnp.where(sub + t == 0, -1e9 / SCALE, a)
                lg.append(a)
            m = lg[0]
            for w in range(1, W):
                m = jnp.maximum(m, lg[w])
            e = [jnp.exp2((a - m) * (SCALE * LOG2E)) for a in lg]
            den = e[0]
            for w in range(1, W):
                den = den + e[w]
            inv = 1.0 / den
            probs[j] = [a * inv for a in e]

        def pv(j):
            p = [ch.after(a) for a in probs.pop(j)]
            for c in range(NC):
                o = p[0] * kv(2 * NC + c, j)
                for w in range(1, W):
                    o = o + p[w] * kv(2 * NC + c, j - w * DIL)
                    if w == W // 2 - 1 and c == NC - 1:
                        ch.mark(o)
                of[c, j * NS:(j + 1) * NS, :] = o

        def combine(j, c):
            r = j * NS

            def ov(cc, rr):
                return [of[cc, pl.ds(rr + i, NS, stride=2), :] for i in range(2)]
            ops = left_operands([ch.after(a) for a in ov(c, r)], ov(c + HC, r),
                                ov(c, r + HM), [ch.after(a) for a in ov(c + HC, r + HM)])
            for m, a in enumerate(ops):
                dst[m, r // 2:r // 2 + 8, lanes(c)] = a
            ch.mark(ops[-1])

        js = [j + o for j in range(0, TJ // 2, 2) for o in (0, 1, TJ // 2, TJ // 2 + 1)]

        jobs = []
        for i in range(TJ + LAG):
            if i < TJ:
                jobs.append((CQ, part(qk, js[i])))
            if i >= LAG:
                jobs.append((CP, part(pv, js[i - LAG])))
                if (i - LAG) % 4 == 3:
                    jobs += [(CC, part(combine, js[i - LAG - 3], c)) for c in range(HC)]
        return jobs

    def emit(mxu, *job_lists, chains=()):
        nm = len(mxu)
        slots = [[] for _ in range(nm)]
        for first, last, jobs in job_lists:
            jobs = [f if isinstance(f, tuple) else (60, f) for f in jobs]
            total, done = sum(cost for cost, _ in jobs), 0
            for cost, f in jobs:
                slots[first + (done * (last - first)) // total].append(f)
                done += cost
        del issued[:]
        for i in range(nm):
            if slots[i] and issued:
                for ch in chains:
                    ch.mark(issued[-1])
            for f in slots[i]:
                f()
            mxu[i]()

    def tile_of(n, off):
        return (n // NT + n % NT + off) % NT

    def slot_of(tau, par):
        if par:
            return (qkv1, 0)
        first = 1 + (tau // NT) % 2
        if isinstance(tau, int):
            return (qkv0, first if tau % NT == 0 else 0)
        return (qkv0, jnp.where(tau % NT == 0, first, 0))

    def step(tau, par, ch, parts=(0, 1, 2), do_proj=True, pre=None, extra=(), xch=()):
        mxu = [f for p in parts
               for f in qkv_jobs((hs[par], (tau // 2) % 4), (tau // NT) % 2, p, slot_of(tau, par))]
        if do_proj:
            mxu += proj_jobs(os_[1 - par], ((tau - 3) // NT) % 2, tile_of(tau - 3, 1))
        if pre is None:
            pre = ln_jobs(tile_of(tau - 5, 1), (hs[1 - par], ((tau + 3) // 2) % 4), ch)
        at = tile_of(tau - 2, 1)
        if par and isinstance(tau, int):
            cur = slot_of(tau - 9 if tau % NT == 1 else tau - 1, 0)
        elif par:
            cur = slot_of(jnp.where(tau % NT == 1, tau - 9, tau - 1), 0)
        else:
            cur = slot_of(tau - 1, 1)
        clamp_halo(at, cur, halos[par])
        vec = pre + attn_jobs(at, cur, halos[par], os_[par], ch)
        nxt = halo_jobs(tile_of(tau - 1, 1), slot_of(tau - 1, 1 - par), halos[1 - par])
        end = len(mxu) * CUT // 56
        emit(mxu, *[(0, end, jobs) for jobs in (vec, nxt, list(extra)) if jobs], chains=[ch] + list(xch))

    zero_ref[0] = 0
    x_copy(0).start()
    x_copy(1).start()
    for i in range(NQD):
        wq_first_copy(i).start()

    free = Chain(on=False)
    for _, f in x_jobs(0, free):
        f()

    per = HD // 2 // NQD

    def wq_head(i, carry):
        wq_first_copy(i).wait()

        @pl.when(i == 1)
        def _():
            for cp in (wq_copy(0, 1), x_copy(2)):
                cp.start()
        rows = [pl.multiple_of(i * per + r2, 8) for r2 in range(0, per, 8)]
        for a in range(NC):
            shuffle_lanes(0, 0, a, rows, free)
        for r2 in rows:
            prep_wq(0, 0, r2, free)
        return carry
    jax.lax.fori_loop(0, NQD, wq_head, 0)

    ch, wch = Chain(), Chain()

    def first(*parts):
        return [f for t, p in parts for f in qkv_jobs(h_of(t), 0, p, slot_of(t, t % 2))]
    emit(first((0, 0)), (0, 22, x_jobs(1, ch)), chains=[ch])
    start_now(wq_copy(0, 2), x_copy(3))
    emit(first((1, 0), (2, 0)), (0, 22, x_jobs(2, ch)), (0, 50, wq_jobs(0, 1, wch)), chains=[ch, wch])
    start_now(wo_copy(0), x_copy(4))
    emit(first((0, 1), (1, 1)), (0, 56, x_jobs(3, ch)), (0, 50, wq_jobs(0, 2, wch)), chains=[ch, wch])
    start_now(wq_copy(1, 0), x_copy(5))
    emit(first((0, 2), (1, 2)), (0, 56, x_jobs(4, ch)), (0, 56, wo_jobs(0, wch)), chains=[ch, wch])
    start_now(wq_copy(1, 1), x_copy(6))
    for f in halo_jobs(tile_of(0, 1), slot_of(0, 0), halos[0]):
        f()
    step(2, 0, ch, parts=(1, 2), do_proj=False, pre=x_jobs(5, ch))
    start_now(wq_copy(1, 2), wo_copy(1), x_copy(7))
    step(3, 1, ch, pre=x_jobs(6, ch), extra=wq_jobs(1, 0, wch) + wq_jobs(1, 1, wch), xch=[wch])
    step(4, 0, ch, pre=x_jobs(7, ch), extra=wq_jobs(1, 2, wch) + wo_jobs(1, wch), xch=[wch])

    def main(i, carry):
        ch = Chain()
        step(2 * i + 1, 1, ch)
        step(2 * i + 2, 0, ch)

        @pl.when(2 * i - 2 >= (NL - 1) * NT)
        def _():
            write_out(tile_of(2 * i - 2, 1))
            write_out(tile_of(2 * i - 1, 1))
        return carry
    last = NL * NT
    jax.lax.fori_loop(2, last // 2 - 1, main, 0)

    ch = Chain()
    n = last - 1
    mxu = [f for p in range(3) for f in qkv_jobs(h_of(n), (NL - 1) % 2, p, slot_of(n, 1))]
    nq = len(mxu)
    for m, src in zip(range(n - 3, n + 1), (os0, os1, os2, os0)):
        mxu += proj_jobs(src, (NL - 1) % 2, tile_of(m, 1))
    npj = (len(mxu) - nq) // 4
    att = []
    for m, cur, dst, g in ((n - 2, slot_of(n - 1, 0), os1, 1), (n - 1, slot_of(n, 1), os2, 2),
                           (n, slot_of(n - 7, 0), os0, 2)):
        t = tile_of(m, 1)
        att.append([part(clamp_halo, t, cur, halos[m % 2])] + attn_jobs(t, cur, halos[m % 2], dst, ch, g))
    outs = [(nq + (i + 1) * npj, nq + (i + 1) * npj + 1, [part(write_out, tile_of(n - 3 + i, 1))])
            for i in range(3)]
    emit(mxu,
         (0, nq, halo_jobs(tile_of(n - 1, 1), slot_of(n - 1, 0), halos[0])), (0, nq, att[0]),
         (nq, nq + npj, halo_jobs(tile_of(n, 1), slot_of(n, 1), halos[1])),
         (nq, nq + 3 * npj, att[1] + att[2]), *outs, chains=[ch])
    write_out(tile_of(n, 1))
    for t in range(NT):
        out_copy(t).wait()


@jax.jit
def pallas_interleave_layers__sliding_local_dilated__sliding_local_dilated__prompt_kernel(
    A_x: jax.Array,
    A_wqkv: jax.Array,
    A_wo: jax.Array,
    B_x: jax.Array,
    B_wqkv: jax.Array,
    B_wo: jax.Array,
):
    del B_x
    f32, bf16, u32 = jnp.float32, jnp.bfloat16, jnp.uint32
    any_spec = pl.BlockSpec(memory_space=pl.ANY)
    out = pl.pallas_call(
        _kernel,
        out_shape=jax.ShapeDtypeStruct((NS, SJ, D), bf16),
        in_specs=[any_spec] * 5,
        out_specs=any_spec,
        scratch_shapes=[
            pltpu.VMEM((NC, S + NS, 128), f32),
            pltpu.VMEM((4, 7, HM // 2, HD), u32),
            pltpu.VMEM((4, 7, HM // 2, HD), u32),
            pltpu.VMEM((3, 3 * NC, TM, 128), f32),
            pltpu.VMEM((1, 3 * NC, TM, 128), f32),
            pltpu.VMEM((2 * NC, HJ * NS, 128), f32),
            pltpu.VMEM((2 * NC, HJ * NS, 128), f32),
            pltpu.VMEM((NC, TM + NS, 128), f32),
            pltpu.VMEM((7, HM // 2, HD), u32),
            pltpu.VMEM((7, HM // 2, HD), u32),
            pltpu.VMEM((7, HM // 2, HD), u32),
            pltpu.VMEM((2, 7, HD // 2, 3 * HD), u32),
            pltpu.VMEM((2, 7, HD // 2, HD), u32),
            pltpu.VMEM((2, 3, 2, HD, D), bf16),
            pltpu.VMEM((2, D, D), bf16),
            pltpu.VMEM((NT, NS, TJ, D), bf16),
            pltpu.VMEM((2, 2, HD // 2, D), u32),
            pltpu.VMEM((2, 2, D + NS, 128), f32),
            pltpu.VMEM((NT, NS, TJ, D), bf16),
            pltpu.SMEM((1,), jnp.int32),
            pltpu.SemaphoreType.DMA((NT,)),
            pltpu.SemaphoreType.DMA((8,)),
            pltpu.SemaphoreType.DMA((NQD,)),
            pltpu.SemaphoreType.DMA((NT,)),
        ],
        compiler_params=pltpu.CompilerParams(vmem_limit_bytes=110 * 2**20),
    )(A_x.reshape(NS, SJ, D), A_wqkv.reshape(2, HD, 3 * D), A_wo, B_wqkv.reshape(2, HD, 3 * D), B_wo)
    return out.reshape(1, S, D)
```
